```python
import os as _os
_os.environ.setdefault("JAX_PLATFORMS", "cpu")
import jax
import jax.numpy as jnp

def _softmax(x, axis=-1):
    return jax.nn.softmax(x, axis=axis)
def _gelu(x):
    return jax.nn.gelu(x, approximate=True)
def _silu(x):
    return jax.nn.silu(x)
def _sigmoid(x):
    return jax.nn.sigmoid(x)
def _layernorm(x, axis=-1, eps=1e-5):
    m = jnp.mean(x, axis=axis, keepdims=True)
    v = jnp.var(x, axis=axis, keepdims=True)
    return (x - m) / jnp.sqrt(v + eps)
def _scatter_add(tgt, idx, src, axis=0):
    return tgt.at[idx].add(src)
def _segment_sum(src, seg, n):
    return jax.ops.segment_sum(src, seg, n)
class _Rng:
    def __init__(self, key):
        self._k = key
    def _next(self):
        self._k, sub = jax.random.split(self._k)
        return sub
    def normal(self, shape):
        return jax.random.normal(self._next(), shape, dtype=jnp.bfloat16)
    def randint(self, lo, hi, shape):
        return jax.random.randint(self._next(), shape, lo, hi, dtype=jnp.int32)
    def uniform(self, shape, lo=0.0, hi=1.0):
        return jax.random.uniform(self._next(), shape, jnp.bfloat16, lo, hi)
    def permutation(self, n):
        return jax.random.permutation(self._next(), n)


kernel_name = 'parallel_sum__sliding_block__moe_arch_mod__prompt'

def setup_inputs():
    _rng = _Rng(jax.random.key(int.from_bytes(__import__("os").urandom(4), "little")))
    _w = (lambda a: (lambda t: t.astype(jnp.bfloat16) if jnp.issubdtype(t.dtype, jnp.floating) else t)(jnp.asarray(a)))
    def _A_setup():
        B, S, D = 1, 2048, 512
        return {
            "x": _w((lambda *s: _rng.normal(s) * 0.05)(B, S, D)),
            "wqkv": _w((lambda *s: _rng.normal(s) * 0.05)(D, 3 * D)),
            "wo": _w((lambda *s: _rng.normal(s) * 0.05)(D, D)),
        }
    _A_in = _A_setup()

    def _B_setup():
        B, S, D, F, C = 1, 2048, 512, 1376, 1
        return {
            "x": _w((lambda *s: _rng.normal(s) * 0.05)(B, S, D)),
            "w_r": _w((lambda *s: _rng.normal(s) * 0.05)(D)),
            "w_gate": _w((lambda *s: _rng.normal(s) * 0.05)(D, F)),
            "w_up": _w((lambda *s: _rng.normal(s) * 0.05)(D, F)),
            "w_down": _w((lambda *s: _rng.normal(s) * 0.05)(F, D)),
        }
    _B_in = _B_setup()

    return {
        "A_x": _A_in["x"],
        "A_wqkv": _A_in["wqkv"],
        "A_wo": _A_in["wo"],
        "B_x": _B_in["x"],
        "B_w_r": _B_in["w_r"],
        "B_w_gate": _B_in["w_gate"],
        "B_w_up": _B_in["w_up"],
        "B_w_down": _B_in["w_down"],
    }

def reference(A_x, A_wqkv, A_wo, B_x, B_w_r, B_w_gate, B_w_up, B_w_down):
    def _A_ref(x, wqkv, wo):
        B, S, D = x.shape
        H = 32; Dh = D // H; W = 256
        qkv = (lambda x, *d: x.transpose(*d))((x @ wqkv).reshape(B, S, 3, H, Dh), 2, 0, 3, 1, 4)
        q, k, v = qkv[0], qkv[1], qkv[2]
        scores = jnp.einsum("bhqd,bhkd->bhqk", q, k) * (Dh ** -0.5)
        idx = jnp.arange(S)
        mask = (idx[:, None] - idx[None, :] >= 0) & (idx[:, None] - idx[None, :] < W)
        scores = jnp.where(mask[None, None], scores, -1e9)
        p = _softmax(scores, axis=-1)
        o = jnp.einsum("bhqk,bhkd->bhqd", p, v)
        return (lambda x, *d: x.transpose(*d))(o, 0, 2, 1, 3).reshape(B, S, D) @ wo

    def _B_ref(x, w_r, w_gate, w_up, w_down):
        B, S, D = x.shape
        C = 1
        r = x @ w_r
        idx = jnp.argsort(-r, axis=-1)[:, :C]
        idx_e = jnp.repeat(idx.reshape(B, C, 1), D, axis=2)
        x_sel = jnp.take_along_axis(x, idx_e, axis=1)
        g = _silu(x_sel @ w_gate)
        u = x_sel @ w_up
        y = (g * u) @ w_down
        r_sel = _sigmoid(jnp.take_along_axis(r, idx, axis=1))
        y = y * r_sel.reshape(B, C, 1)
        b_off = (jnp.arange(B) * S).reshape(B, 1)
        flat_idx = (idx + b_off).reshape(B * C)
        zero = (x * 0.0).reshape(B * S, D)
        upd = _scatter_add(zero, flat_idx, y.reshape(B * C, D), axis=0)
        return x + upd.reshape(B, S, D)

    x = A_x
    xn = _layernorm(x, axis=-1)
    return x + _A_ref(xn, A_wqkv, A_wo) + _B_ref(xn, B_w_r, B_w_gate, B_w_up, B_w_down)
```

```python
import jax
import jax.numpy as jnp
from jax import lax
import jax.experimental.pallas as pl
import jax.experimental.pallas.tpu as pltpu

S = 2048
D = 512
H = 32
DH = D // H
W = 256
F = 1376
TQ = 128
NB = S // TQ
PAD = W
NEG = -1e9
EPS = 1e-5

f32 = jnp.float32
bf16 = jnp.bfloat16


def _kernel(x_ref, wqvT_ref, wk_ref, wo_ref, wr_ref, wg_hbm, wu_hbm, wd_hbm,
            o_ref,
            xn_s, k_s, vt_s, ot_s, wg_v, wu_v, wd_v, sems, idx_s, rbest_s):
    step = pl.program_id(0)

    def ffn_copies():
        return (pltpu.make_async_copy(wg_hbm, wg_v, sems.at[0]),
                pltpu.make_async_copy(wu_hbm, wu_v, sems.at[1]),
                pltpu.make_async_copy(wd_hbm, wd_v, sems.at[2]))

    @pl.when(step == 0)
    def _():
        for cp in ffn_copies():
            cp.start()
        k_s[0:PAD, :] = jnp.zeros((PAD, D), bf16)
        vt_s[:, 0:PAD] = jnp.zeros((D, PAD), bf16)
        wr = wr_ref[...].astype(f32)
        rows = lax.broadcasted_iota(jnp.int32, (TQ, 1), 0)

        def body(c, carry):
            best, idx = carry
            r0 = pl.multiple_of(c * TQ, TQ)
            xf = x_ref[pl.ds(r0, TQ), :].astype(f32)
            mu = jnp.mean(xf, axis=-1, keepdims=True)
            xc = xf - mu
            var = jnp.mean(xc * xc, axis=-1, keepdims=True)
            xnb = (xc / jnp.sqrt(var + EPS)).astype(bf16)
            xn_s[pl.ds(r0, TQ), :] = xnb
            r = jnp.sum(xnb.astype(f32) * wr, axis=-1, keepdims=True)
            r = r.astype(bf16).astype(f32)
            m = jnp.max(r)
            il = jnp.min(jnp.where(r == m, rows, jnp.int32(2 ** 30)))
            better = m > best
            best = jnp.where(better, m, best)
            idx = jnp.where(better, c * TQ + il, idx)
            return best, idx

        best, idx = lax.fori_loop(0, NB, body, (jnp.float32(-jnp.inf), jnp.int32(0)))
        idx_s[0] = idx
        rbest_s[0] = best

    q0 = pl.multiple_of(step * TQ, TQ)
    xn_b = xn_s[pl.ds(q0, TQ), :]
    qvt = lax.dot_general(wqvT_ref[...], xn_b, (((1,), (1,)), ((), ())),
                          preferred_element_type=f32)
    qT = (qvt[0:D].astype(bf16).astype(f32)) * (DH ** -0.5)
    vt_s[:, pl.ds(pl.multiple_of(q0 + PAD, TQ), TQ)] = qvt[D:2 * D].astype(bf16)
    k_s[pl.ds(pl.multiple_of(q0 + PAD, TQ), TQ), :] = jnp.dot(
        xn_b, wk_ref[...], preferred_element_type=f32).astype(bf16)

    r_i = lax.broadcasted_iota(jnp.int32, (TQ, TQ), 0)
    c_i = lax.broadcasted_iota(jnp.int32, (TQ, TQ), 1)
    tri = r_i <= c_i
    hrow = lax.broadcasted_iota(jnp.int32, (128, TQ), 0)

    def attend(use1, use2):
        starts = []
        if use1:
            starts.append(0)
        if use2:
            starts.append(1)
        starts.append(2)
        nrows = TQ * len(starts)
        kbase = pl.multiple_of(q0 + TQ * starts[0], TQ)
        for g in range(D // 128):
            Kg = k_s[pl.ds(kbase, nrows), 128 * g:128 * (g + 1)]
            qTg = qT[128 * g:128 * (g + 1)]
            for hh in range(128 // DH):
                h = g * (128 // DH) + hh
                hm = (hrow >= DH * hh) & (hrow < DH * (hh + 1))
                qTm = jnp.where(hm, qTg, 0.0).astype(bf16)
                s = jnp.dot(Kg, qTm, preferred_element_type=f32)
                off = 0
                if use1:
                    s1 = s[0:TQ]
                    off = TQ
                else:
                    s1 = None
                if use2:
                    s2 = s[off:off + TQ]
                    off += TQ
                s3 = s[off:off + TQ]
                c = jnp.where(tri, s3, s1 if use1 else NEG)
                if use2:
                    m = jnp.max(jnp.maximum(c, s2), axis=0, keepdims=True)
                else:
                    m = jnp.max(c, axis=0, keepdims=True)
                pc = jnp.exp(c - m)
                l = jnp.sum(pc, axis=0, keepdims=True)
                vrows = slice(DH * h, DH * (h + 1))
                p3 = jnp.where(tri, pc, 0.0).astype(bf16)
                o = jnp.dot(vt_s[vrows, pl.ds(pl.multiple_of(q0 + 2 * TQ, TQ), TQ)], p3,
                            preferred_element_type=f32)
                if use1:
                    p1 = jnp.where(tri, 0.0, pc).astype(bf16)
                    o = o + jnp.dot(vt_s[vrows, pl.ds(q0, TQ)], p1,
                                    preferred_element_type=f32)
                if use2:
                    p2 = jnp.exp(s2 - m)
                    l = l + jnp.sum(p2, axis=0, keepdims=True)
                    o = o + jnp.dot(vt_s[vrows, pl.ds(pl.multiple_of(q0 + TQ, TQ), TQ)],
                                    p2.astype(bf16), preferred_element_type=f32)
                ot_s[vrows, :] = (o / l).astype(bf16)

    @pl.when(step == 0)
    def _():
        attend(False, False)

    @pl.when(step == 1)
    def _():
        attend(False, True)

    @pl.when(step >= 2)
    def _():
        attend(True, True)

    attn = lax.dot_general(ot_s[...], wo_ref[...], (((0,), (0,)), ((), ())),
                           preferred_element_type=f32)
    xn_f = xn_b.astype(f32)
    base = x_ref[pl.ds(q0, TQ), :].astype(f32) + attn + xn_f
    o_ref[...] = base.astype(o_ref.dtype)

    idx = idx_s[0]

    @pl.when(idx // TQ == step)
    def _():
        for cp in ffn_copies():
            cp.wait()
        sel = lax.broadcasted_iota(jnp.int32, (TQ, 1), 0) == (idx - q0)
        x_sel = jnp.sum(jnp.where(sel, xn_f, 0.0), axis=0, keepdims=True)
        x_sel = jnp.broadcast_to(x_sel, (8, D)).astype(bf16)
        gt = jnp.dot(x_sel, wg_v[...], preferred_element_type=f32)
        u = jnp.dot(x_sel, wu_v[...], preferred_element_type=f32)
        hcur = (gt * jax.nn.sigmoid(gt)) * u
        y = jnp.dot(hcur.astype(bf16), wd_v[...], preferred_element_type=f32)
        y = y[0:1] * jax.nn.sigmoid(rbest_s[0])
        o_ref[...] = (base + jnp.where(sel, y, 0.0)).astype(o_ref.dtype)


@jax.jit
def pallas_parallel_sum__sliding_block__moe_arch_mod__prompt_kernel(
    A_x: jax.Array,
    A_wqkv: jax.Array,
    A_wo: jax.Array,
    B_x: jax.Array,
    B_w_r: jax.Array,
    B_w_gate: jax.Array,
    B_w_up: jax.Array,
    B_w_down: jax.Array,
):
    del B_x
    x = A_x.reshape(S, D)
    wqvT = jnp.concatenate([A_wqkv[:, 0:D].T, A_wqkv[:, 2 * D:3 * D].T], axis=0)
    wk = A_wqkv[:, D:2 * D]
    wr = B_w_r.reshape(1, D)

    const = lambda i: (0, 0)
    out = pl.pallas_call(
        _kernel,
        grid=(NB,),
        in_specs=[
            pl.BlockSpec((S, D), const),
            pl.BlockSpec((2 * D, D), const),
            pl.BlockSpec((D, D), const),
            pl.BlockSpec((D, D), const),
            pl.BlockSpec((1, D), const),
            pl.BlockSpec(memory_space=pl.ANY),
            pl.BlockSpec(memory_space=pl.ANY),
            pl.BlockSpec(memory_space=pl.ANY),
        ],
        out_specs=pl.BlockSpec((TQ, D), lambda i: (i, 0)),
        out_shape=jax.ShapeDtypeStruct((S, D), A_x.dtype),
        scratch_shapes=[
            pltpu.VMEM((S, D), bf16),
            pltpu.VMEM((S + PAD, D), bf16),
            pltpu.VMEM((D, S + PAD), bf16),
            pltpu.VMEM((D, TQ), bf16),
            pltpu.VMEM((D, F), bf16),
            pltpu.VMEM((D, F), bf16),
            pltpu.VMEM((F, D), bf16),
            pltpu.SemaphoreType.DMA((3,)),
            pltpu.SMEM((1,), jnp.int32),
            pltpu.SMEM((1,), f32),
        ],
        compiler_params=pltpu.CompilerParams(
            dimension_semantics=("arbitrary",),
            vmem_limit_bytes=64 * 1024 * 1024),
    )(x, wqvT, wk, A_wo, wr, B_w_gate, B_w_up, B_w_down)
    return out.reshape(1, S, D)
```

```python
import jax
import jax.numpy as jnp
from jax import lax
import jax.experimental.pallas as pl
import jax.experimental.pallas.tpu as pltpu

S = 2048
D = 512
H = 32
DH = D // H
W = 256
F = 1376
TQ = 128
NB = S // TQ
XCH = 512
TB = 512
SUB = TB // TQ
NSTEP = S // TB
PAD = W
NEG = -1e9
EPS = 1e-5
LOOKAHEAD = 4

f32 = jnp.float32
bf16 = jnp.bfloat16


def _kernel(x_hbm, wqkv_hbm, wo_hbm, wr_ref, wg_hbm, wu_hbm, wd_hbm,
            o_ref,
            x_ref, wqkv_ref, wo_ref, xn_s, k_s, vt_s, qt_s, ot_s, wg_v, wu_v, wd_v, sems, idx_s, rbest_s):
    step = pl.program_id(0)

    def ffn_copies():
        return (pltpu.make_async_copy(wg_hbm, wg_v, sems.at[0]),
                pltpu.make_async_copy(wu_hbm, wu_v, sems.at[1]),
                pltpu.make_async_copy(wd_hbm, wd_v, sems.at[2]))

    def w_copies():
        return (pltpu.make_async_copy(wqkv_hbm, wqkv_ref, sems.at[3]),
                pltpu.make_async_copy(wo_hbm, wo_ref, sems.at[4]))

    def x_copy(c):
        rows = pl.ds(c * XCH, XCH)
        return pltpu.make_async_copy(x_hbm.at[rows, :], x_ref.at[rows, :], sems.at[5 + c])

    @pl.when(step == 0)
    def _():
        for c in range(S // XCH):
            x_copy(c).start()
        for cp in w_copies():
            cp.start()
        k_s[0:PAD, :] = jnp.zeros((PAD, D), bf16)
        vt_s[:, 0:PAD] = jnp.zeros((D, PAD), bf16)
        wr = wr_ref[...].astype(f32)
        rows = lax.broadcasted_iota(jnp.int32, (TQ, 1), 0)

        def body(c, carry):
            best, idx = carry
            r0 = pl.multiple_of(c * TQ, TQ)
            xf = x_ref[pl.ds(r0, TQ), :].astype(f32)
            mu = jnp.mean(xf, axis=-1, keepdims=True)
            xc = xf - mu
            var = jnp.mean(xc * xc, axis=-1, keepdims=True)
            xnb = (xc / jnp.sqrt(var + EPS)).astype(bf16)
            xn_s[pl.ds(r0, TQ), :] = xnb
            r = jnp.sum(xnb.astype(f32) * wr, axis=-1, keepdims=True)
            r = r.astype(bf16).astype(f32)
            m = jnp.max(r)
            il = jnp.min(jnp.where(r == m, rows, jnp.int32(2 ** 30)))
            better = m > best
            best = jnp.where(better, m, best)
            idx = jnp.where(better, c * TQ + il, idx)
            return best, idx

        best, idx = jnp.float32(-jnp.inf), jnp.int32(0)
        cpb = XCH // TQ
        for c in range(S // XCH):
            x_copy(c).wait()
            best, idx = lax.fori_loop(c * cpb, (c + 1) * cpb, body, (best, idx), unroll=cpb)
        for cp in ffn_copies():
            cp.start()
        for cp in w_copies():
            cp.wait()
        idx_s[0] = idx
        rbest_s[0] = best

    b0 = pl.multiple_of(step * TB, TB)
    xn_b = xn_s[pl.ds(b0, TB), :]
    qkv = jnp.dot(xn_b, wqkv_ref[...], preferred_element_type=f32)
    qt_s[...] = (qkv[:, 0:D].astype(bf16).astype(f32) * (DH ** -0.5)).T
    vt_s[:, pl.ds(pl.multiple_of(b0 + PAD, TQ), TB)] = qkv[:, 2 * D:3 * D].T.astype(bf16)
    k_s[pl.ds(pl.multiple_of(b0 + PAD, TQ), TB), :] = qkv[:, D:2 * D].astype(bf16)

    r_i = lax.broadcasted_iota(jnp.int32, (TQ, TQ), 0)
    c_i = lax.broadcasted_iota(jnp.int32, (TQ, TQ), 1)
    tri = r_i <= c_i
    hrow = lax.broadcasted_iota(jnp.int32, (128, TQ), 0)

    def attend(q0, qc, use1, use2):
        tiles = ([0] if use1 else []) + ([1] if use2 else []) + [2]

        def koff(t):
            return pl.multiple_of(q0 + TQ * t, TQ)

        def scores(h):
            g, hh = divmod(h, 128 // DH)
            hm = (hrow >= DH * hh) & (hrow < DH * (hh + 1))
            qTm = jnp.where(hm, qt_s[128 * g:128 * (g + 1), pl.ds(qc, TQ)], 0.0).astype(bf16)
            return {t: jnp.dot(k_s[pl.ds(koff(t), TQ), 128 * g:128 * (g + 1)], qTm,
                               preferred_element_type=f32) for t in tiles}

        def finish(h, s):
            vrows = slice(DH * h, DH * (h + 1))
            c = jnp.where(tri, s[2], s[0] if use1 else NEG)
            if use2:
                m = jnp.max(jnp.maximum(c, s[1]), axis=0, keepdims=True)
            else:
                m = jnp.max(c, axis=0, keepdims=True)
            pc = jnp.exp(c - m)
            l = jnp.sum(pc, axis=0, keepdims=True)
            p = {2: jnp.where(tri, pc, 0.0).astype(bf16)}
            if use1:
                p[0] = jnp.where(tri, 0.0, pc).astype(bf16)
            if use2:
                p2 = jnp.exp(s[1] - m)
                l = l + jnp.sum(p2, axis=0, keepdims=True)
                p[1] = p2.astype(bf16)
            o = None
            for t in tiles:
                d = jnp.dot(vt_s[vrows, pl.ds(koff(t), TQ)], p[t], preferred_element_type=f32)
                o = d if o is None else o + d
            ot_s[vrows, pl.ds(qc, TQ)] = (o / l).astype(bf16)

        pending = [scores(h) for h in range(LOOKAHEAD)]
        for h in range(H):
            if h + LOOKAHEAD < H:
                pending.append(scores(h + LOOKAHEAD))
            finish(h, pending.pop(0))

    def sub_block(j, carry):
        qc = pl.multiple_of(j * TQ, TQ)
        q0 = pl.multiple_of(b0 + qc, TQ)

        @pl.when(q0 == 0)
        def _():
            attend(q0, qc, False, False)

        @pl.when(q0 == TQ)
        def _():
            attend(q0, qc, False, True)

        @pl.when(q0 >= 2 * TQ)
        def _():
            attend(q0, qc, True, True)
        return carry

    lax.fori_loop(0, SUB, sub_block, 0)

    attn = lax.dot_general(ot_s[...], wo_ref[...], (((0,), (0,)), ((), ())),
                           preferred_element_type=f32)
    xn_f = xn_b.astype(f32)
    base = x_ref[pl.ds(b0, TB), :].astype(f32) + attn + xn_f
    o_ref[...] = base.astype(o_ref.dtype)

    idx = idx_s[0]

    @pl.when(idx // TB == step)
    def _():
        for cp in ffn_copies():
            cp.wait()
        sel = lax.broadcasted_iota(jnp.int32, (TB, 1), 0) == (idx - b0)
        x_sel = jnp.sum(jnp.where(sel, xn_f, 0.0), axis=0, keepdims=True)
        x_sel = jnp.broadcast_to(x_sel, (8, D)).astype(bf16)
        nt = (((1,), (1,)), ((), ()))
        gt = lax.dot_general(x_sel, wg_v[...], nt, preferred_element_type=f32)
        u = lax.dot_general(x_sel, wu_v[...], nt, preferred_element_type=f32)
        hcur = (gt * jax.nn.sigmoid(gt)) * u
        y = jnp.dot(hcur.astype(bf16), wd_v[...], preferred_element_type=f32)
        y = y[0:1] * jax.nn.sigmoid(rbest_s[0])
        o_ref[...] = (base + jnp.where(sel, y, 0.0)).astype(o_ref.dtype)


@jax.jit
def pallas_parallel_sum__sliding_block__moe_arch_mod__prompt_kernel(
    A_x: jax.Array,
    A_wqkv: jax.Array,
    A_wo: jax.Array,
    B_x: jax.Array,
    B_w_r: jax.Array,
    B_w_gate: jax.Array,
    B_w_up: jax.Array,
    B_w_down: jax.Array,
):
    del B_x
    x = A_x.reshape(S, D)
    wr = B_w_r.reshape(1, D)

    const = lambda i: (0, 0)
    out = pl.pallas_call(
        _kernel,
        grid=(NSTEP,),
        in_specs=[
            pl.BlockSpec(memory_space=pl.ANY),
            pl.BlockSpec(memory_space=pl.ANY),
            pl.BlockSpec(memory_space=pl.ANY),
            pl.BlockSpec((1, D), const),
            pl.BlockSpec(memory_space=pl.ANY),
            pl.BlockSpec(memory_space=pl.ANY),
            pl.BlockSpec(memory_space=pl.ANY),
        ],
        out_specs=pl.BlockSpec((TB, D), lambda i: (i, 0)),
        out_shape=jax.ShapeDtypeStruct((S, D), A_x.dtype),
        scratch_shapes=[
            pltpu.VMEM((S, D), bf16),
            pltpu.VMEM((D, 3 * D), bf16),
            pltpu.VMEM((D, D), bf16),
            pltpu.VMEM((S, D), bf16),
            pltpu.VMEM((S + PAD, D), bf16),
            pltpu.VMEM((D, S + PAD), bf16),
            pltpu.VMEM((D, TB), f32),
            pltpu.VMEM((D, TB), bf16),
            pltpu.VMEM((F, D), bf16),
            pltpu.VMEM((F, D), bf16),
            pltpu.VMEM((F, D), bf16),
            pltpu.SemaphoreType.DMA((5 + S // XCH,)),
            pltpu.SMEM((1,), jnp.int32),
            pltpu.SMEM((1,), f32),
        ],
        compiler_params=pltpu.CompilerParams(
            dimension_semantics=("arbitrary",),
            vmem_limit_bytes=64 * 1024 * 1024),
    )(x, A_wqkv, A_wo, wr, B_w_gate.T, B_w_up.T, B_w_down)
    return out.reshape(1, S, D)
```
